```python
import os as _os
_os.environ.setdefault("JAX_PLATFORMS", "cpu")
import jax
import jax.numpy as jnp

def _softmax(x, axis=-1):
    return jax.nn.softmax(x, axis=axis)
def _gelu(x):
    return jax.nn.gelu(x, approximate=True)
def _silu(x):
    return jax.nn.silu(x)
def _sigmoid(x):
    return jax.nn.sigmoid(x)
def _layernorm(x, axis=-1, eps=1e-5):
    m = jnp.mean(x, axis=axis, keepdims=True)
    v = jnp.var(x, axis=axis, keepdims=True)
    return (x - m) / jnp.sqrt(v + eps)
def _scatter_add(tgt, idx, src, axis=0):
    return tgt.at[idx].add(src)
def _segment_sum(src, seg, n):
    return jax.ops.segment_sum(src, seg, n)
class _Rng:
    def __init__(self, key):
        self._k = key
    def _next(self):
        self._k, sub = jax.random.split(self._k)
        return sub
    def normal(self, shape):
        return jax.random.normal(self._next(), shape, dtype=jnp.bfloat16)
    def randint(self, lo, hi, shape):
        return jax.random.randint(self._next(), shape, lo, hi, dtype=jnp.int32)
    def uniform(self, shape, lo=0.0, hi=1.0):
        return jax.random.uniform(self._next(), shape, jnp.bfloat16, lo, hi)
    def permutation(self, n):
        return jax.random.permutation(self._next(), n)


kernel_name = 'gated_mix__ssm_conv_s5__geglu_ffn__prompt'

def setup_inputs():
    _rng = _Rng(jax.random.key(int.from_bytes(__import__("os").urandom(4), "little")))
    _w = (lambda a: (lambda t: t.astype(jnp.bfloat16) if jnp.issubdtype(t.dtype, jnp.floating) else t)(jnp.asarray(a)))
    def _A_setup():
        B, S, D = 1, 2048, 512
        P = D
        Lambda_re = -0.5 * jnp.exp((lambda *s: _rng.normal(s) * 0.4)(P))
        Lambda_im = (lambda *s: _rng.normal(s) * 0.4)(P) * 1.0
        B_re = (lambda *s: _rng.normal(s) * 0.4)(P, D) * (D ** -0.5)
        B_im = (lambda *s: _rng.normal(s) * 0.4)(P, D) * (D ** -0.5)
        C_re = (lambda *s: _rng.normal(s) * 0.4)(D, P) * (P ** -0.5)
        C_im = (lambda *s: _rng.normal(s) * 0.4)(D, P) * (P ** -0.5)
        log_dt = (lambda *s: _rng.normal(s) * 0.4)(P) * 0.3 - 2.0
        Dskip = (lambda *s: _rng.normal(s) * 0.4)(D)
        return {
            "x": _w((lambda *s: _rng.normal(s) * 0.05)(B, S, D)),
            "Lambda_re": _w(Lambda_re),
            "Lambda_im": _w(Lambda_im),
            "B_re": _w(B_re),
            "B_im": _w(B_im),
            "C_re": _w(C_re),
            "C_im": _w(C_im),
            "log_dt": _w(log_dt),
            "Dskip": _w(Dskip),
        }
    _A_in = _A_setup()

    def _B_setup():
        B, S, D, F = 1, 2048, 512, 1376
        return {
            "x": _w((lambda *s: _rng.normal(s) * 0.05)(B, S, D)),
            "w_gate": _w((lambda *s: _rng.normal(s) * 0.1)(D, F)),
            "w_up": _w((lambda *s: _rng.normal(s) * 0.1)(D, F)),
            "w_down": _w((lambda *s: _rng.normal(s) * 0.1)(F, D)),
        }
    _B_in = _B_setup()

    return {
        "A_x": _A_in["x"],
        "A_Lambda_re": _A_in["Lambda_re"],
        "A_Lambda_im": _A_in["Lambda_im"],
        "A_B_re": _A_in["B_re"],
        "A_B_im": _A_in["B_im"],
        "A_C_re": _A_in["C_re"],
        "A_C_im": _A_in["C_im"],
        "A_log_dt": _A_in["log_dt"],
        "A_Dskip": _A_in["Dskip"],
        "B_x": _B_in["x"],
        "B_w_gate": _B_in["w_gate"],
        "B_w_up": _B_in["w_up"],
        "B_w_down": _B_in["w_down"],
        "gate_w": _w((lambda *s: _rng.normal(s) * 0.05)(512) * 16.0),
    }

def reference(A_x, A_Lambda_re, A_Lambda_im, A_B_re, A_B_im, A_C_re, A_C_im, A_log_dt, A_Dskip, B_x, B_w_gate, B_w_up, B_w_down, gate_w):
    def _A_ref(x, Lambda_re, Lambda_im, B_re, B_im, C_re, C_im, log_dt, Dskip):
        Bsz, L, H = x.shape
        Lam = Lambda_re + 1j * Lambda_im
        Bmat = B_re + 1j * B_im
        Cmat = C_re + 1j * C_im
        dt = jnp.exp(log_dt)
        Lam_bar = jnp.exp(dt * Lam)
        B_bar = ((Lam_bar - 1.0) / Lam)[:, None] * Bmat
        Bu = jnp.einsum("bld,pd->blp", x + 0j, B_bar)
        h = jnp.zeros_like(Bu[:, 0, :])
        hs = []
        for t in range(L):
            h = Lam_bar[None, :] * h + Bu[:, t, :]
            hs.append(h)
        hseq = jnp.stack(hs, 1)
        y = 2.0 * jnp.einsum("blp,dp->bld", hseq, Cmat).real + x * Dskip[None, None, :]
        return y

    def _B_ref(x, w_gate, w_up, w_down):
        return (_gelu(x @ w_gate) * (x @ w_up)) @ w_down

    x = A_x
    g = _sigmoid((x * gate_w).sum(-1, keepdims=True))
    a = _A_ref(x, A_Lambda_re, A_Lambda_im, A_B_re, A_B_im, A_C_re, A_C_im, A_log_dt, A_Dskip)
    b = _B_ref(x, B_w_gate, B_w_up, B_w_down)
    return g * a + (1 - g) * b
```

```python
import jax
import jax.numpy as jnp
import jax.experimental.pallas as pl
import jax.experimental.pallas.tpu as pltpu

TM = 512
NSEG = 8
T = TM // NSEG
_NT = (((1,), (1,)), ((), ()))


def _lam(lre, lim, ldt):
    dt = jnp.exp(ldt)
    mag = jnp.exp(dt * lre)
    ang = dt * lim
    return mag * jnp.cos(ang), mag * jnp.sin(ang)


def _kernel(x_ref, lre_r, lim_r, ldt_r, lre_c, lim_c, ldt_c, bre_ref, bim_ref,
            cre_ref, cim_ref, dskip_ref, wg_ref, wu_ref, wd_ref, gw_ref,
            o_ref, bcat, ccat, lam_s, pw, carry, bu, hin):
    P = bre_ref.shape[0]
    f32 = jnp.float32

    @pl.when(pl.program_id(0) == 0)
    def _init():
        lr = lre_c[...].astype(f32)
        li = lim_c[...].astype(f32)
        ar, ai = _lam(lr, li, ldt_c[...].astype(f32))
        nr = ar - 1.0
        den = lr * lr + li * li
        cr = (nr * lr + ai * li) / den
        ci = (ai * lr - nr * li) / den
        br = bre_ref[...].astype(f32)
        bi = bim_ref[...].astype(f32)
        bcat[0:P, :] = (cr * br - ci * bi).astype(bcat.dtype)
        bcat[P:2 * P, :] = (cr * bi + ci * br).astype(bcat.dtype)
        ccat[:, 0:P] = cre_ref[...] * 2.0
        ccat[:, P:2 * P] = cim_ref[...] * -2.0
        ar, ai = _lam(lre_r[...].astype(f32), lim_r[...].astype(f32),
                      ldt_r[...].astype(f32))
        ar8 = jnp.broadcast_to(ar, (NSEG, P))
        ai8 = jnp.broadcast_to(ai, (NSEG, P))
        lam_s[:, 0:P] = ar8
        lam_s[:, P:2 * P] = ai8

        def pbody(j, c):
            pr, pi = c
            pw[j, :, 0:P] = pr
            pw[j, :, P:2 * P] = pi
            return pr * ar8 - pi * ai8, pr * ai8 + pi * ar8
        jax.lax.fori_loop(0, T, pbody, (ar8, ai8))
        carry[...] = jnp.zeros(carry.shape, f32)

    xb = x_ref[0]
    NC = 2 * P // 128
    xB = jax.lax.dot_general(xb, bcat[...], _NT, preferred_element_type=f32)
    for k in range(NC):
        bu[k] = xB[:, k * 128:(k + 1) * 128]

    def ld(j):
        return jnp.concatenate(
            [bu[k, pl.ds(j, NSEG, stride=T), :] for k in range(NC)], axis=1)

    def st(j, nr, ni):
        v = jnp.concatenate([nr, ni], axis=1)
        for k in range(NC):
            bu[k, pl.ds(j, NSEG, stride=T), :] = v[:, k * 128:(k + 1) * 128]

    ar = lam_s[:, 0:P]
    ai = lam_s[:, P:2 * P]

    def scan(j, c):
        hr, hi = c
        v = ld(j)
        nr = ar * hr - ai * hi + v[:, 0:P]
        ni = ar * hi + ai * hr + v[:, P:2 * P]
        st(j, nr, ni)
        return nr, ni
    z = jnp.zeros((NSEG, P), f32)
    er, ei = jax.lax.fori_loop(0, T, scan, (z, z), unroll=8)

    tr = pw[T - 1, 0:1, 0:P]
    ti = pw[T - 1, 0:1, P:2 * P]
    cr = carry[0:1, 0:P]
    ci = carry[0:1, P:2 * P]
    for s in range(NSEG):
        hin[s:s + 1, 0:P] = cr
        hin[s:s + 1, P:2 * P] = ci
        cr, ci = (er[s:s + 1] + tr * cr - ti * ci,
                  ei[s:s + 1] + tr * ci + ti * cr)
    carry[0:1, 0:P] = cr
    carry[0:1, P:2 * P] = ci
    Hr = hin[:, 0:P]
    Hi = hin[:, P:2 * P]

    def fix(j, _):
        v = ld(j)
        p = pw[j]
        pr = p[:, 0:P]
        pi = p[:, P:2 * P]
        nr = v[:, 0:P] + pr * Hr - pi * Hi
        ni = v[:, P:2 * P] + pr * Hi + pi * Hr
        st(j, nr, ni)
        return 0
    jax.lax.fori_loop(0, T, fix, 0, unroll=8)

    xf = xb.astype(f32)
    a = jax.lax.dot_general(
        jnp.concatenate([bu[k].astype(jnp.bfloat16) for k in range(NC)], axis=1), ccat[...], _NT,
                            preferred_element_type=f32)
    a = a + xf * dskip_ref[...].astype(f32)

    gt = jnp.dot(xb, wg_ref[...], preferred_element_type=f32)
    up = jnp.dot(xb, wu_ref[...], preferred_element_type=f32)
    act = (jax.nn.gelu(gt, approximate=True) * up).astype(jnp.bfloat16)
    b = jnp.dot(act, wd_ref[...], preferred_element_type=f32)

    g = jax.nn.sigmoid(jnp.sum(xf * gw_ref[...].astype(f32), axis=-1,
                               keepdims=True))
    o_ref[0] = g * a + (1.0 - g) * b


@jax.jit
def pallas_gated_mix__ssm_conv_s5__geglu_ffn__prompt_kernel(
    A_x, A_Lambda_re, A_Lambda_im, A_B_re, A_B_im, A_C_re, A_C_im, A_log_dt,
    A_Dskip, B_x, B_w_gate, B_w_up, B_w_down, gate_w,
):
    _, L, D = A_x.shape
    P = A_B_re.shape[0]
    F = B_w_gate.shape[1]
    row = lambda v: v.reshape(1, -1)
    col = lambda v: v.reshape(-1, 1)
    full = lambda s: pl.BlockSpec(s, lambda i: (0,) * len(s))
    f32 = jnp.float32
    return pl.pallas_call(
        _kernel,
        grid=(L // TM,),
        in_specs=[pl.BlockSpec((1, TM, D), lambda i: (0, i, 0))]
        + [full((1, P))] * 3 + [full((P, 1))] * 3
        + [full((P, D))] * 2 + [full((D, P))] * 2 + [full((1, D))]
        + [full((D, F))] * 2 + [full((F, D)), full((1, D))],
        out_specs=pl.BlockSpec((1, TM, D), lambda i: (0, i, 0)),
        out_shape=jax.ShapeDtypeStruct((1, L, D), f32),
        scratch_shapes=[
            pltpu.VMEM((2 * P, D), jnp.bfloat16),
            pltpu.VMEM((D, 2 * P), jnp.bfloat16),
            pltpu.VMEM((NSEG, 2 * P), f32),
            pltpu.VMEM((T, NSEG, 2 * P), f32),
            pltpu.VMEM((1, 2 * P), f32),
            pltpu.VMEM((2 * P // 128, TM, 128), f32),
            pltpu.VMEM((NSEG, 2 * P), f32),
        ],
        compiler_params=pltpu.CompilerParams(
            dimension_semantics=("arbitrary",),
            vmem_limit_bytes=96 * 1024 * 1024),
    )(A_x, row(A_Lambda_re), row(A_Lambda_im), row(A_log_dt),
      col(A_Lambda_re), col(A_Lambda_im), col(A_log_dt),
      A_B_re, A_B_im, A_C_re, A_C_im, row(A_Dskip),
      B_w_gate, B_w_up, B_w_down, row(gate_w))
```

```python
import jax
import jax.numpy as jnp
import jax.experimental.pallas as pl
import jax.experimental.pallas.tpu as pltpu

TM = 512
NSEG = 8
T = TM // NSEG
_NT = (((1,), (1,)), ((), ()))


def _lam(lre, lim, ldt):
    dt = jnp.exp(ldt)
    mag = jnp.exp(dt * lre)
    ang = dt * lim
    return mag * jnp.cos(ang), mag * jnp.sin(ang)


def _kernel(x_ref, lre_r, lim_r, ldt_r, bre_ref, bim_ref,
            cre_ref, cim_ref, dskip_ref, wg_ref, wu_ref, wd_ref, gw_ref,
            o_ref, bcat, ccat, lam_s, pw, carry, bu, hin):
    P = bre_ref.shape[0]
    f32 = jnp.float32

    @pl.when(pl.program_id(0) == 0)
    def _init():
        lr = lre_r[...].astype(f32).reshape(1, P)
        li = lim_r[...].astype(f32).reshape(1, P)
        ar, ai = _lam(lr, li, ldt_r[...].astype(f32).reshape(1, P))
        nr = ar - 1.0
        den = lr * lr + li * li
        cr = (nr * lr + ai * li) / den
        ci = (ai * lr - nr * li) / den
        bcat[0:P, :] = bre_ref[...]
        bcat[P:2 * P, :] = bim_ref[...]
        c_r = cre_ref[...].astype(f32)
        c_i = cim_ref[...].astype(f32)
        ccat[:, 0:P] = (2.0 * (c_r * cr - c_i * ci)).astype(ccat.dtype)
        ccat[:, P:2 * P] = (-2.0 * (c_r * ci + c_i * cr)).astype(ccat.dtype)
        ar8 = jnp.broadcast_to(ar, (NSEG, P))
        ai8 = jnp.broadcast_to(ai, (NSEG, P))
        row = jax.lax.broadcasted_iota(jnp.int32, (NSEG, P), 0)
        pr, pi = ar8, ai8
        tr, ti = ar8, ai8
        for e in range(1, NSEG + 1):
            if e in (1, 2, 4):
                k = (1, 2, 4).index(e)
                pw[k, :, 0:P] = jnp.where(row >= e, pr, 0.0)
                pw[k, :, P:2 * P] = jnp.where(row >= e, pi, 0.0)
            tr = jnp.where(row == e - 1, pr, tr)
            ti = jnp.where(row == e - 1, pi, ti)
            pr, pi = pr * ar8 - pi * ai8, pr * ai8 + pi * ar8
        pw[3, :, 0:P] = tr
        pw[3, :, P:2 * P] = ti
        carry[...] = jnp.zeros(carry.shape, f32)

    xb = x_ref[0]
    bu[...] = jax.lax.dot_general(xb, bcat[...], _NT, preferred_element_type=f32)

    def tile(i, c):
        cr, ci = c
        r0 = pl.multiple_of(i * NSEG, NSEG)
        vr = bu[pl.ds(r0, NSEG), 0:P]
        vi = bu[pl.ds(r0, NSEG), P:2 * P]
        for k in range(3):
            mr = pw[k, :, 0:P]
            mi = pw[k, :, P:2 * P]
            sr = pltpu.roll(vr, 1 << k, 0)
            si = pltpu.roll(vi, 1 << k, 0)
            vr, vi = vr + mr * sr - mi * si, vi + mr * si + mi * sr
        mr = pw[3, :, 0:P]
        mi = pw[3, :, P:2 * P]
        vr, vi = vr + mr * cr - mi * ci, vi + mr * ci + mi * cr
        bu[pl.ds(r0, NSEG), 0:P] = vr
        bu[pl.ds(r0, NSEG), P:2 * P] = vi
        return (jnp.broadcast_to(vr[NSEG - 1:NSEG], (NSEG, P)),
                jnp.broadcast_to(vi[NSEG - 1:NSEG], (NSEG, P)))
    c0 = (jnp.broadcast_to(carry[0:1, 0:P], (NSEG, P)),
          jnp.broadcast_to(carry[0:1, P:2 * P], (NSEG, P)))
    cr, ci = jax.lax.fori_loop(0, TM // NSEG, tile, c0, unroll=4)
    carry[0:1, 0:P] = cr[0:1]
    carry[0:1, P:2 * P] = ci[0:1]

    xf = xb.astype(f32)
    a = jax.lax.dot_general(bu[...].astype(jnp.bfloat16), ccat[...], _NT,
                            preferred_element_type=f32)
    a = a + xf * dskip_ref[...].astype(f32).reshape(1, -1)

    gt = jax.lax.dot_general(xb, wg_ref[...], _NT, preferred_element_type=f32)
    up = jax.lax.dot_general(xb, wu_ref[...], _NT, preferred_element_type=f32)
    act = (jax.nn.gelu(gt, approximate=True) * up).astype(jnp.bfloat16)
    b = jnp.dot(act, wd_ref[...], preferred_element_type=f32)

    g = jax.nn.sigmoid(jnp.sum(xf * gw_ref[...].astype(f32).reshape(1, -1), axis=-1,
                               keepdims=True))
    o_ref[0] = g * a + (1.0 - g) * b


@jax.jit
def pallas_gated_mix__ssm_conv_s5__geglu_ffn__prompt_kernel(
    A_x, A_Lambda_re, A_Lambda_im, A_B_re, A_B_im, A_C_re, A_C_im, A_log_dt,
    A_Dskip, B_x, B_w_gate, B_w_up, B_w_down, gate_w,
):
    _, L, D = A_x.shape
    P = A_B_re.shape[0]
    F = B_w_gate.shape[1]
    row = lambda v: v.reshape(1, -1)
    col = lambda v: v.reshape(-1, 1)
    full = lambda s: pl.BlockSpec(s, lambda i: (0,) * len(s))
    f32 = jnp.float32
    return pl.pallas_call(
        _kernel,
        grid=(L // TM,),
        in_specs=[pl.BlockSpec((1, TM, D), lambda i: (0, i, 0))]
        + [full((P,))] * 3
        + [full((P, D))] * 2 + [full((D, P))] * 2 + [full((D,))]
        + [full((F, D))] * 3 + [full((D,))],
        out_specs=pl.BlockSpec((1, TM, D), lambda i: (0, i, 0)),
        out_shape=jax.ShapeDtypeStruct((1, L, D), f32),
        scratch_shapes=[
            pltpu.VMEM((2 * P, D), jnp.bfloat16),
            pltpu.VMEM((D, 2 * P), jnp.bfloat16),
            pltpu.VMEM((NSEG, 2 * P), f32),
            pltpu.VMEM((4, NSEG, 2 * P), f32),
            pltpu.VMEM((1, 2 * P), f32),
            pltpu.VMEM((TM, 2 * P), f32),
            pltpu.VMEM((NSEG, 2 * P), f32),
        ],
        compiler_params=pltpu.CompilerParams(
            dimension_semantics=("arbitrary",),
            vmem_limit_bytes=96 * 1024 * 1024),
    )(A_x, A_Lambda_re, A_Lambda_im, A_log_dt,
      A_B_re, A_B_im, A_C_re, A_C_im, A_Dskip,
      B_w_gate.T, B_w_up.T, B_w_down, gate_w)
```

```python
import jax
import jax.numpy as jnp
import jax.experimental.pallas as pl
import jax.experimental.pallas.tpu as pltpu

TM = 512
NSEG = 8
T = TM // NSEG
_NT = (((1,), (1,)), ((), ()))


def _lam(lre, lim, ldt):
    dt = jnp.exp(ldt)
    mag = jnp.exp(dt * lre)
    ang = dt * lim
    return mag * jnp.cos(ang), mag * jnp.sin(ang)


def _kernel(x_ref, lre_r, lim_r, ldt_r, bre_ref, bim_ref,
            cre_ref, cim_ref, dskip_ref, wg_ref, wu_ref, wd_ref, gw_ref,
            o_ref, bcat, ccat, pw, carry, bu):
    P = bre_ref.shape[0]
    f32 = jnp.float32

    @pl.when(pl.program_id(0) == 0)
    def _init():
        lr = lre_r[...].astype(f32).reshape(1, P)
        li = lim_r[...].astype(f32).reshape(1, P)
        ar, ai = _lam(lr, li, ldt_r[...].astype(f32).reshape(1, P))
        nr = ar - 1.0
        den = lr * lr + li * li
        cr = (nr * lr + ai * li) / den
        ci = (ai * lr - nr * li) / den
        bcat[0:P, :] = bre_ref[...]
        bcat[P:2 * P, :] = bim_ref[...]
        c_r = cre_ref[...].astype(f32)
        c_i = cim_ref[...].astype(f32)
        ccat[:, 0:P] = (2.0 * (c_r * cr - c_i * ci)).astype(ccat.dtype)
        ccat[:, P:2 * P] = (-2.0 * (c_r * ci + c_i * cr)).astype(ccat.dtype)
        ar8 = jnp.broadcast_to(ar, (NSEG, P))
        ai8 = jnp.broadcast_to(ai, (NSEG, P))
        row = jax.lax.broadcasted_iota(jnp.int32, (NSEG, P), 0)
        pr, pi = ar8, ai8
        tr, ti = ar8, ai8
        for e in range(1, NSEG + 1):
            if e in (1, 2, 4):
                k = (1, 2, 4).index(e)
                pw[k, :, 0:P] = jnp.where(row >= e, pr, 0.0)
                pw[k, :, P:2 * P] = jnp.where(row >= e, pi, 0.0)
            tr = jnp.where(row == e - 1, pr, tr)
            ti = jnp.where(row == e - 1, pi, ti)
            pr, pi = pr * ar8 - pi * ai8, pr * ai8 + pi * ar8
        pw[3, :, 0:P] = tr
        pw[3, :, P:2 * P] = ti
        carry[...] = jnp.zeros(carry.shape, f32)

    xb = x_ref[0]
    bu[...] = jax.lax.dot_general(xb, bcat[...], _NT, preferred_element_type=f32)

    def tile(i, c):
        cr, ci = c
        r0 = pl.multiple_of(i * NSEG, NSEG)
        vr = bu[pl.ds(r0, NSEG), 0:P]
        vi = bu[pl.ds(r0, NSEG), P:2 * P]
        for k in range(3):
            mr = pw[k, :, 0:P]
            mi = pw[k, :, P:2 * P]
            sr = pltpu.roll(vr, 1 << k, 0)
            si = pltpu.roll(vi, 1 << k, 0)
            vr, vi = vr + mr * sr - mi * si, vi + mr * si + mi * sr
        mr = pw[3, :, 0:P]
        mi = pw[3, :, P:2 * P]
        vr, vi = vr + mr * cr - mi * ci, vi + mr * ci + mi * cr
        bu[pl.ds(r0, NSEG), 0:P] = vr
        bu[pl.ds(r0, NSEG), P:2 * P] = vi
        return (jnp.broadcast_to(vr[NSEG - 1:NSEG], (NSEG, P)),
                jnp.broadcast_to(vi[NSEG - 1:NSEG], (NSEG, P)))
    c0 = (jnp.broadcast_to(carry[0:1, 0:P], (NSEG, P)),
          jnp.broadcast_to(carry[0:1, P:2 * P], (NSEG, P)))
    cr, ci = jax.lax.fori_loop(0, TM // NSEG, tile, c0, unroll=4)
    carry[0:1, 0:P] = cr[0:1]
    carry[0:1, P:2 * P] = ci[0:1]

    xf = xb.astype(f32)
    a = jax.lax.dot_general(bu[...].astype(jnp.bfloat16), ccat[...], _NT,
                            preferred_element_type=f32)
    a = a + xf * dskip_ref[...].astype(f32).reshape(1, -1)

    gt = jax.lax.dot_general(xb, wg_ref[...], _NT, preferred_element_type=f32)
    up = jax.lax.dot_general(xb, wu_ref[...], _NT, preferred_element_type=f32)
    act = (jax.nn.gelu(gt, approximate=True) * up).astype(jnp.bfloat16)
    b = jnp.dot(act, wd_ref[...], preferred_element_type=f32)

    g = jax.nn.sigmoid(jnp.sum(xf * gw_ref[...].astype(f32).reshape(1, -1), axis=-1,
                               keepdims=True))
    o_ref[0] = g * a + (1.0 - g) * b


@jax.jit
def pallas_gated_mix__ssm_conv_s5__geglu_ffn__prompt_kernel(
    A_x, A_Lambda_re, A_Lambda_im, A_B_re, A_B_im, A_C_re, A_C_im, A_log_dt,
    A_Dskip, B_x, B_w_gate, B_w_up, B_w_down, gate_w,
):
    _, L, D = A_x.shape
    P = A_B_re.shape[0]
    F = B_w_gate.shape[1]
    full = lambda s: pl.BlockSpec(s, lambda i: (0,) * len(s))
    f32 = jnp.float32
    return pl.pallas_call(
        _kernel,
        grid=(L // TM,),
        in_specs=[pl.BlockSpec((1, TM, D), lambda i: (0, i, 0))]
        + [full((P,))] * 3
        + [full((P, D))] * 2 + [full((D, P))] * 2 + [full((D,))]
        + [full((F, D))] * 3 + [full((D,))],
        out_specs=pl.BlockSpec((1, TM, D), lambda i: (0, i, 0)),
        out_shape=jax.ShapeDtypeStruct((1, L, D), f32),
        scratch_shapes=[
            pltpu.VMEM((2 * P, D), jnp.bfloat16),
            pltpu.VMEM((D, 2 * P), jnp.bfloat16),
            pltpu.VMEM((4, NSEG, 2 * P), f32),
            pltpu.VMEM((1, 2 * P), f32),
            pltpu.VMEM((TM, 2 * P), f32),
        ],
        compiler_params=pltpu.CompilerParams(
            dimension_semantics=("arbitrary",),
            vmem_limit_bytes=96 * 1024 * 1024),
    )(A_x, A_Lambda_re, A_Lambda_im, A_log_dt,
      A_B_re, A_B_im, A_C_re, A_C_im, A_Dskip,
      B_w_gate.T, B_w_up.T, B_w_down, gate_w)
```
